```python
import os as _os
_os.environ.setdefault("JAX_PLATFORMS", "cpu")
import jax
import jax.numpy as jnp

def _softmax(x, axis=-1):
    return jax.nn.softmax(x, axis=axis)
def _gelu(x):
    return jax.nn.gelu(x, approximate=True)
def _silu(x):
    return jax.nn.silu(x)
def _sigmoid(x):
    return jax.nn.sigmoid(x)
def _layernorm(x, axis=-1, eps=1e-5):
    m = jnp.mean(x, axis=axis, keepdims=True)
    v = jnp.var(x, axis=axis, keepdims=True)
    return (x - m) / jnp.sqrt(v + eps)
def _scatter_add(tgt, idx, src, axis=0):
    return tgt.at[idx].add(src)
def _segment_sum(src, seg, n):
    return jax.ops.segment_sum(src, seg, n)
class _Rng:
    def __init__(self, key):
        self._k = key
    def _next(self):
        self._k, sub = jax.random.split(self._k)
        return sub
    def normal(self, shape):
        return jax.random.normal(self._next(), shape, dtype=jnp.bfloat16)
    def randint(self, lo, hi, shape):
        return jax.random.randint(self._next(), shape, lo, hi, dtype=jnp.int32)
    def uniform(self, shape, lo=0.0, hi=1.0):
        return jax.random.uniform(self._next(), shape, jnp.bfloat16, lo, hi)
    def permutation(self, n):
        return jax.random.permutation(self._next(), n)


kernel_name = 'concat_heads__grouped_kv_mqa__sliding_block__prompt'

def setup_inputs():
    _rng = _Rng(jax.random.key(int.from_bytes(__import__("os").urandom(4), "little")))
    _w = (lambda a: (lambda t: t.astype(jnp.bfloat16) if jnp.issubdtype(t.dtype, jnp.floating) else t)(jnp.asarray(a)))
    def _A_setup():
        B, S, D, H = 1, 2048, 576, 32
        Dh = D // H
        return {
            "x": _w((lambda *s: _rng.normal(s) * 0.05)(B, S, D)),
            "wq": _w((lambda *s: _rng.normal(s) * 1.6)(D, H * Dh)),
            "wk": _w((lambda *s: _rng.normal(s) * 1.6)(D, Dh)),
            "wv": _w((lambda *s: _rng.normal(s) * 0.1)(D, Dh)),
            "wo": _w((lambda *s: _rng.normal(s) * 0.1)(H * Dh, D)),
        }
    _A_in = _A_setup()

    def _B_setup():
        B, S, D = 1, 2048, 576
        return {
            "x": _w((lambda *s: _rng.normal(s) * 0.2)(B, S, D)),
            "wqkv": _w((lambda *s: _rng.normal(s) * 0.2)(D, 3 * D)),
            "wo": _w((lambda *s: _rng.normal(s) * 0.05)(D, D)),
        }
    _B_in = _B_setup()

    return {
        "A_x": _A_in["x"],
        "A_wq": _A_in["wq"],
        "A_wk": _A_in["wk"],
        "A_wv": _A_in["wv"],
        "A_wo": _A_in["wo"],
        "B_x": _B_in["x"],
        "B_wqkv": _B_in["wqkv"],
        "B_wo": _B_in["wo"],
    }

def reference(A_x, A_wq, A_wk, A_wv, A_wo, B_x, B_wqkv, B_wo):
    def _A_ref(x, wq, wk, wv, wo):
        B, S, D = x.shape
        H = 32
        Dh = D // H
        q = (lambda x, *d: x.transpose(*d))((x @ wq).reshape(B, S, H, Dh), 0, 2, 1, 3)
        k = x @ wk
        v = x @ wv
        scores = jnp.einsum("bhqd,bkd->bhqk", q, k) * (Dh ** -0.5)
        p = _softmax(scores, axis=-1)
        o = jnp.einsum("bhqk,bkd->bhqd", p, v)
        return (lambda x, *d: x.transpose(*d))(o, 0, 2, 1, 3).reshape(B, S, H * Dh) @ wo

    def _B_ref(x, wqkv, wo):
        B, S, D = x.shape
        H = 32; Dh = D // H; W = 256
        qkv = (lambda x, *d: x.transpose(*d))((x @ wqkv).reshape(B, S, 3, H, Dh), 2, 0, 3, 1, 4)
        q, k, v = qkv[0], qkv[1], qkv[2]
        scores = jnp.einsum("bhqd,bhkd->bhqk", q, k) * (Dh ** -0.5)
        idx = jnp.arange(S)
        mask = (idx[:, None] - idx[None, :] >= 0) & (idx[:, None] - idx[None, :] < W)
        scores = jnp.where(mask[None, None], scores, -1e9)
        p = _softmax(scores, axis=-1)
        o = jnp.einsum("bhqk,bhkd->bhqd", p, v)
        return (lambda x, *d: x.transpose(*d))(o, 0, 2, 1, 3).reshape(B, S, D) @ wo

    a = _A_ref(A_x, A_wq, A_wk, A_wv, A_wo)
    b = _B_ref(B_x, B_wqkv, B_wo)
    return jnp.concatenate([a, b], axis=-1)
```

```python
import math

import jax
import jax.numpy as jnp
from jax import lax
import jax.experimental.pallas as pl
import jax.experimental.pallas.tpu as pltpu

S = 2048
D = 576
H = 32
DH = D // H
WINDOW = 256

T = 128
QB = 512
NQ = S // QB
HP = 32
VP = 24
A_UNROLL = 4
B_HEADS = 4

F32 = jnp.float32
BF16 = jnp.bfloat16
QSCALE = DH**-0.5 * math.log2(math.e)

assert WINDOW == 2 * T


def _dot(a, b):
    return lax.dot_general(a, b, (((1,), (0,)), ((), ())), preferred_element_type=F32)


def _pad_rows(x, rows):
    return jnp.concatenate([x, jnp.zeros((rows - x.shape[0], x.shape[1]), x.dtype)], axis=0)


def _v_ext(v):
    n = v.shape[1]
    tail = (lax.broadcasted_iota(jnp.int32, (VP - DH, n), 0) == 0).astype(F32)
    return jnp.concatenate([v.astype(BF16).astype(F32), tail], axis=0)


def _row_max(x):
    return jnp.max(x.reshape(x.shape[0] // 8, 8, x.shape[1]), axis=0)


def _exp2_shifted(s, m):
    r, n = s.shape
    return jnp.exp2(s.reshape(r // 8, 8, n) - m[None]).reshape(r, n)


def _normalize(acc):
    return acc * (1.0 / acc[DH : DH + 1, :])


def _kernel(
    xa_hbm, wq_hbm, wkt_hbm, wvt_hbm, woa_hbm, xb_hbm, wqkv_hbm, wob_hbm,
    out_hbm,
    xa, wq, wkt, wvt, woa, xb, wqkv, wob,
    wat, wbt, woat, wobt,
    qa, ka, va, sa, oa,
    qb, kb, vb, ob,
    obuf, in_sem, out_sem,
):
    def x_copy(src, dst, c, sem):
        return pltpu.make_async_copy(src.at[:, pl.ds(c * QB, QB)], dst.at[c], in_sem.at[sem])

    cp_wq = pltpu.make_async_copy(wq_hbm, wq, in_sem.at[0])
    cp_wk = pltpu.make_async_copy(wkt_hbm, wkt, in_sem.at[1])
    cp_wv = pltpu.make_async_copy(wvt_hbm, wvt, in_sem.at[2])
    cp_xa = [x_copy(xa_hbm, xa, c, 3 + c) for c in range(NQ)]
    cp_wqkv = pltpu.make_async_copy(wqkv_hbm, wqkv, in_sem.at[3 + NQ])
    cp_xb = [x_copy(xb_hbm, xb, c, 4 + NQ + c) for c in range(NQ)]
    cp_woa = pltpu.make_async_copy(woa_hbm, woa, in_sem.at[4 + 2 * NQ])
    cp_wob = pltpu.make_async_copy(wob_hbm, wob, in_sem.at[5 + 2 * NQ])
    for cp in [cp_wq, cp_wk, cp_wv, *cp_xa, cp_wqkv, *cp_xb, cp_woa, cp_wob]:
        cp.start()

    sa[...] = jnp.zeros(sa.shape, F32)

    cp_wq.wait()
    wat[0:D, :] = wq[...].T
    cp_wk.wait()
    cp_wv.wait()
    wkv = jnp.concatenate([wkt[...].astype(F32), wvt[...].astype(F32)], axis=0)
    wat[D:, :] = _pad_rows(wkv, wat.shape[0] - D).astype(BF16)
    for c in range(NQ):
        cp_xa[c].wait()
        r = _dot(wat[...], xa[c])
        for h in range(H):
            qa[c * H + h] = _pad_rows(r[h * DH : (h + 1) * DH] * QSCALE, HP).astype(BF16)
        ka[pl.ds(c * QB, QB), :] = _pad_rows(r[D : D + DH], HP).astype(BF16).T
        va[:, pl.ds(c * QB, QB)] = _v_ext(r[D + DH : D + 2 * DH])

    cp_wqkv.wait()
    wbt[...] = wqkv[...].T
    for c in range(NQ):
        cp_xb[c].wait()
    cp_woa.wait()
    cp_wob.wait()

    def b_proj(c, carry):
        x = xb[c]
        k = _dot(wbt[D : 2 * D, :], x)
        for h in range(H):
            kh = _pad_rows(k[h * DH : (h + 1) * DH], HP).astype(BF16)
            kb[h, pl.ds(pl.multiple_of(c * QB, QB), QB), :] = jnp.concatenate([kh] * 4, axis=0).T
        q = _dot(wbt[0:D, :], x)
        for h in range(H):
            qb[h, c] = _pad_rows(q[h * DH : (h + 1) * DH] * QSCALE, HP).astype(BF16)
        v = _dot(wbt[2 * D :, :], x)
        for h in range(H):
            vb[h, c] = _v_ext(v[h * DH : (h + 1) * DH])
        return carry

    lax.fori_loop(0, NQ, b_proj, None)

    woat[...] = woa[...].T
    wobt[...] = wob[...].T

    tpc = QB // T

    def b_attn(g, carry):
        row = lax.broadcasted_iota(jnp.int32, (T, T), 0)
        col = lax.broadcasted_iota(jnp.int32, (T, T), 1)
        causal = row <= col
        slot_of_group = (row // HP) == (col // HP)
        lane = lax.broadcasted_iota(jnp.int32, (HP, T), 1)

        def tile(ref, h, i):
            return ref[h, i // tpc, :, pl.ds((i % tpc) * T, T)]

        def scores(h, i):
            q = tile(qb, h, i)
            w = jnp.where(slot_of_group, jnp.concatenate([q] * 4, axis=0), jnp.zeros((), BF16))
            q0 = i * T
            if i >= 2:
                rows = [kb[h, pl.ds(q0, HP), :]]
                for c in range(1, 4):
                    low = kb[h, pl.ds(q0 - WINDOW + (c - 1) * HP, HP), :]
                    high = kb[h, pl.ds(q0 + c * HP, HP), :]
                    rows.append(jnp.where(lane < c * HP, low, high))
                rows.append(kb[h, pl.ds(q0 - WINDOW + 3 * HP, HP), :])
                z = _dot(jnp.concatenate(rows, axis=0), w)
                tri = jnp.where(causal, z[0:T], z[HP : HP + T])
            else:
                tri = jnp.where(causal, _dot(kb[h, pl.ds(q0, T), :], w), -jnp.inf)
            mid = _dot(kb[h, pl.ds(q0 - T, T), :], w) if i >= 1 else None
            return tri, mid

        def attend(h, i, tri, mid):
            m = _row_max(tri)
            if mid is not None:
                m = jnp.maximum(m, _row_max(mid))
            m = jnp.broadcast_to(jnp.max(m, axis=0, keepdims=True), (8, T))
            p = _exp2_shifted(tri, m)
            if i >= 2:
                acc = _dot(tile(vb, h, i), jnp.where(causal, p, 0.0).astype(BF16))
                acc += _dot(tile(vb, h, i - 2), jnp.where(causal, 0.0, p).astype(BF16))
            else:
                acc = _dot(tile(vb, h, i), p.astype(BF16))
            if mid is not None:
                acc += _dot(tile(vb, h, i - 1), _exp2_shifted(mid, m).astype(BF16))
            ob[h, i // tpc, :, pl.ds((i % tpc) * T, T)] = _normalize(acc)

        heads = [g * B_HEADS + l for l in range(B_HEADS)]
        prev = None
        for i in range(S // T + 1):
            cur = [scores(h, i) for h in heads] if i < S // T else None
            if prev is not None:
                for h, (tri, mid) in zip(heads, prev):
                    attend(h, i - 1, tri, mid)
            prev = cur
        return carry

    lax.fori_loop(0, H // B_HEADS, b_attn, None)

    def a_step(q, m_prev):
        acc = None
        mx = None
        for j in range(S // T):
            keys = pl.ds(j * T, T)
            p = _exp2_shifted(sa[keys, :], m_prev).astype(BF16)
            if q is not None:
                s = _dot(ka[keys, :], q)
                sa[keys, :] = s
                mx = _row_max(s) if mx is None else jnp.maximum(mx, _row_max(s))
            o = _dot(va[:, keys], p)
            acc = o if acc is None else acc + o
        if q is not None:
            mx = jnp.broadcast_to(jnp.max(mx, axis=0, keepdims=True), (8, QB))
        return _normalize(acc), mx

    def a_attn(t, m):
        for u in range(A_UNROLL):
            n = t * A_UNROLL + u
            o, m = a_step(qa[n], m)
            oa[n] = o
        return m

    m = lax.fori_loop(0, NQ * H // A_UNROLL, a_attn, jnp.zeros((8, QB), F32))
    oa[NQ * H] = a_step(None, m)[0]

    def out_copy(c):
        return pltpu.make_async_copy(
            obuf.at[c], out_hbm.at[pl.ds(pl.multiple_of(c * QB, QB), QB), :], out_sem.at[c]
        )

    def out_proj(c, carry):
        ot_b = jnp.concatenate([ob[h, c, 0:DH, :] for h in range(H)], axis=0).astype(BF16)
        ot_a = jnp.concatenate([oa[c * H + h + 1, 0:DH, :] for h in range(H)], axis=0).astype(BF16)
        bt = _dot(wobt[...], ot_b).astype(BF16)
        at = _dot(woat[...], ot_a).astype(BF16)
        obuf[c] = jnp.concatenate([at, bt], axis=0).T
        out_copy(c).start()
        return carry

    lax.fori_loop(0, NQ, out_proj, None)
    for c in range(NQ):
        out_copy(c).wait()


@jax.jit
def pallas_concat_heads__grouped_kv_mqa__sliding_block__prompt_kernel(
    A_x: jax.Array,
    A_wq: jax.Array,
    A_wk: jax.Array,
    A_wv: jax.Array,
    A_wo: jax.Array,
    B_x: jax.Array,
    B_wqkv: jax.Array,
    B_wo: jax.Array,
):
    assert A_x.shape == (1, S, D) and B_x.shape == (1, S, D)
    vmem = pltpu.VMEM
    out = pl.pallas_call(
        _kernel,
        out_shape=jax.ShapeDtypeStruct((S, 2 * D), BF16),
        in_specs=[pl.BlockSpec(memory_space=pl.ANY)] * 8,
        out_specs=pl.BlockSpec(memory_space=pl.ANY),
        scratch_shapes=[
            vmem((NQ, D, QB), BF16),
            vmem((D, D), BF16),
            vmem((DH, D), BF16),
            vmem((DH, D), BF16),
            vmem((D, D), BF16),
            vmem((NQ, D, QB), BF16),
            vmem((D, 3 * D), BF16),
            vmem((D, D), BF16),
            vmem((D + 48, D), BF16),
            vmem((3 * D, D), BF16),
            vmem((D, D), BF16),
            vmem((D, D), BF16),
            vmem((NQ * H, HP, QB), BF16),
            vmem((S, HP), BF16),
            vmem((VP, S), F32),
            vmem((S, QB), F32),
            vmem((NQ * H + 1, VP, QB), F32),
            vmem((H, NQ, HP, QB), BF16),
            vmem((H, S, T), BF16),
            vmem((H, NQ, VP, QB), F32),
            vmem((H, NQ, VP, QB), F32),
            vmem((NQ, QB, 2 * D), BF16),
            pltpu.SemaphoreType.DMA((6 + 2 * NQ,)),
            pltpu.SemaphoreType.DMA((NQ,)),
        ],
        compiler_params=pltpu.CompilerParams(vmem_limit_bytes=112 * 1024 * 1024),
        name="mqa_swa_fused",
    )(A_x[0].T, A_wq, A_wk.T, A_wv.T, A_wo, B_x[0].T, B_wqkv, B_wo)
    return out[None]
```

```python
import functools
import itertools
import math

import jax
import jax.numpy as jnp
from jax import lax
import jax.experimental.pallas as pl
import jax.experimental.pallas.tpu as pltpu

S = 2048
D = 576
H = 32
DH = D // H
WINDOW = 256

T = 128
NT = S // T
NMXU = 4
QB = NMXU * T
NQ = S // QB
KT = pl.cdiv(D, T)
HP = 32
VP = 24
HG = 8
BG = 4

A_PAIRS = NT * H
A_UNROLL = 16
A_LOOP = [48] * 8 + [0] * 8
A_FIRST = [32] * 8 + [0] * 8
A_EARLY = ([0] * NT, [0] * 8 + [16] * 4 + [32] * 4, [0] * NT, [0] * 8 + [32] * 8)
PERIOD = len(A_EARLY)
A_EARLY_MAX = [max(x) for x in zip(*A_EARLY)]
EARLY_A_PROJ = (0, 0, 16, 14)
EARLY_B_PROJ = 48
EARLY_B_FIRST = 26
EARLY_B_PASS = 24
EARLY_OUT = 32

F32 = jnp.float32
BF16 = jnp.bfloat16
U32 = jnp.uint32
QSCALE = DH**-0.5 * math.log2(math.e)

assert WINDOW == 2 * T and A_UNROLL == NT and EARLY_A_PROJ[:2] == (0, 0)
assert all(n % PERIOD == 0 for n in (EARLY_B_PROJ, EARLY_B_PASS, EARLY_OUT))
assert A_PAIRS == (
    sum(EARLY_A_PROJ) + NQ * EARLY_B_PROJ + EARLY_B_FIRST + (H // BG - 1) * EARLY_B_PASS + (NQ - 1) * EARLY_OUT
)


def _dot(a, b):
    return lax.dot_general(a, b, (((1,), (0,)), ((), ())), preferred_element_type=F32)


def _iota(shape, axis):
    return lax.broadcasted_iota(jnp.int32, shape, axis)


def _pack(x):
    return pltpu.bitcast(x.astype(BF16), U32)


def _unpack(x):
    return pltpu.bitcast(x, BF16)


def _rows(ref, start, size):
    return _unpack(ref[pl.ds(start // 2, size // 2), :])


def _pad_rows(x, rows):
    return jnp.concatenate([x, jnp.zeros((rows - x.shape[0], x.shape[1]), x.dtype)], axis=0)


def _round(x):
    return x.astype(BF16).astype(F32)


def _sum(xs):
    return functools.reduce(lambda a, b: a + b, xs)


def _add(acc, x):
    return x if acc is None else acc + x


def _inner(k, q):
    return jnp.sum(jnp.sum((k * q).reshape(-1, 3, 8, T), axis=0), axis=0)


def _splat(x, row):
    return jnp.broadcast_to(x[row : row + 1], (8, T))


def _window(x, head):
    first = head * DH // 8 * 8
    return x[first : first + VP], head * DH - first


def _ones_row(offset):
    return 0 if offset else DH


def _no_check():
    return jnp.zeros((1, T), F32), jnp.zeros((1, T), F32), jnp.zeros((8, T), F32)


def _normalize(acc, row, check):
    total = acc[row : row + 1]
    inv = pltpu.reciprocal(total, approx=True)
    inv = inv * (2.0 - total * inv)
    check[0] = jnp.maximum(check[0], total)
    check[1] = jnp.maximum(check[1], inv)
    return acc * inv


def _unsafe(check):
    total, inv, checksum = check
    safe = (total <= 2.0**110) & (inv <= 2.0**40) & (jnp.abs(checksum) < jnp.inf)
    return jnp.min(jnp.where(safe, 1.0, 0.0)) < 0.5


class _Spread:
    def __init__(self, tasks=(), ticks=0):
        self.queue, self.batch, self.ticks, self.seen = [], [], ticks, 0
        self.add(tasks, 0.0, 1.0)

    def add(self, tasks, start, stop):
        self.queue += [((start + (stop - start) * (i + 0.5) / len(tasks)) * self.ticks, t) for i, t in enumerate(tasks)]
        self.queue.sort(key=lambda entry: entry[0])

    def tick(self, x):
        self.batch.append(x)
        if len(self.batch) < NMXU:
            return
        for r in range(0, max(x.shape[0] for x in self.batch), 8):
            for x in self.batch:
                if r < x.shape[0]:
                    self.seen += 1
                    while self.queue and self.queue[0][0] <= self.seen:
                        self.queue.pop(0)[1](x[r : r + 8])
        self.batch = []

    def finish(self):
        assert self.seen == self.ticks and not self.queue


def _put(dst, value, result):
    dst[...] = jnp.concatenate([result] * (value.shape[0] // 8), axis=0)
    dst[...] = value


def _proj(a, b, spread):
    acc = None
    for k in range(0, a.shape[1], T):
        part = _dot(a[:, k : k + T], b[k : k + T])
        spread.tick(part)
        acc = _add(acc, part)
    return acc


def _kernel(
    xa_hbm, wq_hbm, wkt_hbm, wvt_hbm, woa_hbm, xb_hbm, wqkv_hbm, wob_hbm,
    out_hbm,
    xa, wq, woa, xb, wqkv, wob,
    wqt, wbt, woat, wobt,
    qa, ka, k_early, k_loop, keep, va, pa, pa_early, oa,
    qb, kb, vb, pb, obt,
    obufs, order, wkt, wvt, in_sem, out_sem,
):
    in_sems = itertools.count()

    def fetch(src, dst):
        copy = pltpu.make_async_copy(src, dst, in_sem.at[next(in_sems)])
        copy.start()
        return copy

    def wait(copies):
        for copy in copies:
            copy.wait()

    cp_wq, cp_wk, cp_wv = fetch(wq_hbm, wq), fetch(wkt_hbm, wkt), fetch(wvt_hbm, wvt)
    cp_xa = [fetch(xa_hbm.at[:, pl.ds(c * QB, QB)], xa.at[c]) for c in range(NQ)]
    cp_wqkv = fetch(wqkv_hbm, wqkv)
    cp_xb = [fetch(xb_hbm.at[:, pl.ds(c * QB, QB)], xb.at[c]) for c in range(NQ)]
    cp_wo = [fetch(wob_hbm, wob), fetch(woa_hbm, woa)]

    slots = itertools.count()

    def drain(value, result):
        slot = next(slots) % order.shape[0]
        order[slot] = pltpu.bitcast(value, U32)
        order[slot] = pltpu.bitcast(result[0:8, 0:T], U32)

    def early_row(phase, tile):
        return sum(map(sum, A_EARLY[:phase])) + sum(A_EARLY[phase][:tile])

    def early_tasks(start, offset, count):
        def task(u, q, j, r, result):
            if not q:
                rows = qa[start + offset + u, 0:VP]
                q.append(jnp.stack([_splat(rows, d) for d in range(DH)]))
            at = sum(A_EARLY_MAX[: j + 1]) - A_EARLY[(start + u) % PERIOD][j] + r
            s = _inner(k_early[:, pl.ds(at, 8), :], q[0])
            dst = pl.ds(early_row((start + u) % PERIOD, j) + r, 8)
            _put(pa_early.at[offset // PERIOD + (start + u) // PERIOD, dst, :], jnp.exp2(s), result)

        tasks = []
        for u in range(count):
            q = []
            keys = A_EARLY[(start + u) % PERIOD]
            tasks += [functools.partial(task, u, q, j, r) for j in range(NT) for r in range(0, keys[j], 8)]
        return tasks

    def loop_block(tile, row):
        return (sum(A_LOOP[: tile + 1]) - T + row) // 16

    def halves(d):
        return (d, 8 + d) if d < 8 else (16, 17)

    def loop_tasks(n, u, counts):
        def operands(b11, b21, b12, b22):
            t1 = b12 - b11
            t2 = b22 - t1
            return b11, b21, b22, t2 - b21, t1, t2, b22 - b12

        qs = qa[n, 0:VP], qa[n + 1, 0:VP]
        most = operands(*[q[r : r + 8] for q in qs for r in halves(0)])
        last = operands(*[_splat(q, d) for q in qs for d in halves(8)])
        right = {}

        def product(b, e):
            if e not in right:
                right[e] = jnp.stack([_splat(most[e], d) for d in range(8)] + [last[e]])
            return _inner(k_loop[b, pl.ds(e * (DH // 2), DH // 2)], right[e])

        def step(stage, j, r, result):
            b = loop_block(j, r)
            kept = keep.at[u // 2, b]
            out = lambda pair, half: pa.at[u + pair, pl.ds(j * T + r + 8 * half, 8), :]
            if stage == 0:
                _put(kept.at[0], product(b, 0), result)
            elif stage == 1:
                _put(out(0, 0), jnp.exp2(kept[0] + product(b, 1)), result)
            elif stage == 2:
                _put(kept.at[1], kept[0] + product(b, 5), result)
            elif stage == 3:
                _put(kept.at[2], kept[1] + product(b, 6), result)
            elif stage == 4:
                _put(out(0, 1), jnp.exp2(kept[2] - product(b, 3)), result)
            elif stage == 5:
                p5 = product(b, 4)
                _put(out(1, 1), jnp.exp2(kept[2] + p5), result)
                _put(kept.at[3], kept[1] + p5, result)
            else:
                _put(out(1, 0), jnp.exp2(kept[3] + product(b, 2)), result)

        blocks = [(j, r) for j in range(NT) for r in range(T - counts[j], T, 16)]
        return [functools.partial(step, stage, j, r) for stage in range(7) for j, r in blocks]

    def a_keys(c, kv, center):
        k = _round(_pad_rows(kv[0:DH] - center, HP)).T
        ka[pl.ds(c * QB // 2, QB // 2), :] = _pack(k)
        ones = (_iota((VP - DH, QB), 0) == 0).astype(F32)
        va[:, pl.ds(c * QB, QB)] = jnp.concatenate([kv[DH : 2 * DH], ones], axis=0)

        def column(j, r, d):
            at = j % NMXU * T + r
            return jnp.broadcast_to(k[at : at + 16, d : d + 1], (16, T))

        def early(j, r, d, result):
            x = column(j, r, d)
            k_early[d, pl.ds(sum(A_EARLY_MAX[: j + 1]) - T + r, 16), :] = x
            drain(x[8:16], result)

        def loop(j, r, d, result):
            lo, hi = (column(j, r, e) for e in halves(d))
            a11, a12, a21, a22 = lo[0:8], hi[0:8], lo[8:16], hi[8:16]
            s1 = a21 + a22
            s2 = s1 - a11
            s4 = a12 - s2
            for e, x in enumerate((a11, a12, s4, a22, s1, s2, a11 - a21)):
                k_loop[loop_block(j, r), e * (DH // 2) + d] = x
            drain(s4, result)

        tasks = []
        for j in range(c * NMXU, (c + 1) * NMXU):
            for task, count, width in ((early, A_EARLY_MAX[j], DH), (loop, A_LOOP[j], DH // 2)):
                tasks += [functools.partial(task, j, r, d) for r in range(T - count, T, 16) for d in range(width)]
        return tasks

    def a_queries(i, g, q):
        q = _round(q * QSCALE)
        for l in range(HG):
            qa[i * H + g * HG + l, 0:VP] = _pad_rows(q[l * DH : (l + 1) * DH], VP)

    cp_wq.wait()
    wqt[...] = _pack(wq[...].T)
    wait([cp_wk, cp_wv, cp_xa[0]])
    wkv = _pad_rows(jnp.concatenate([wkt[...].astype(F32), wvt[...].astype(F32)], axis=0), 40)
    kv = _dot(wkv, xa[0])
    center = jnp.mean(kv[0:DH], axis=1, keepdims=True)
    for c in range(NQ):
        spread = _Spread(early_tasks(sum(EARLY_A_PROJ[:c]), 0, EARLY_A_PROJ[c]), D // 8 * NMXU * KT)
        if c == 0:
            spread.add(a_keys(0, kv, center), 0.2, 1.0)
        elif c == 1:
            spread.add([t for e in range(1, NQ) for t in a_keys(e, _dot(wkv, xa[e]), center)], 0.0, 1.0)
        for i in range(NMXU):
            for g in range(H // HG):
                q = _proj(_rows(wqt, g * HG * DH, HG * DH), xa[c, :, pl.ds(i * T, T)], spread)
                if (i, g) == (NMXU - 1, H // HG - 1):
                    wait((cp_xa[1:], [], [cp_wqkv], cp_xb)[c])
                    if c == NQ - 2:
                        wbt[...] = _pack(wqkv[...].T)
                a_queries(c * NMXU + i, g, q)
        spread.finish()

    def b_proj(c, carry):
        x = xb[c]
        row = _iota((VP, T), 0)
        early = early_tasks(sum(EARLY_A_PROJ), c * EARLY_B_PROJ, EARLY_B_PROJ)
        spread = _Spread(early, 3 * D // 8 * NMXU * KT)
        for i in range(0, NMXU, 2):
            for g in range(H // HG):

                def proj(e, base):
                    return _proj(_rows(wbt, base + g * HG * DH, HG * DH), x[:, e * T : (e + 1) * T], spread)

                ks = []
                for e in (i, i + 1):
                    k = proj(e, D)
                    q = proj(e, 0) * QSCALE
                    for l in range(HG):
                        qh, at = _window(q, l)
                        qh = jnp.where((row >= at) & (row < at + DH), qh, 0.0)
                        own = jnp.sum((qh * _window(k, l)[0]).reshape(VP // 8, 8, T), axis=0)
                        qb[g * HG + l, c * NMXU + e] = _pack(jnp.concatenate([qh, own], axis=0))
                    ks.append(k)
                k = jnp.concatenate(ks, axis=1)
                for l in range(HG):
                    kh = jnp.concatenate([_window(k, l)[0], jnp.full((HP - VP, 2 * T), -1.0, F32)], axis=0)
                    at = pl.multiple_of(c * (QB // 2), QB // 2) + i * T // 2
                    kb[g * HG + l, pl.ds(at, T), :] = _pack(jnp.concatenate([kh] * 4, axis=0).astype(BF16).T)
                for e in (i, i + 1):
                    v = proj(e, 2 * D)
                    for l in range(HG):
                        vh, at = _window(v, l)
                        vb[g * HG + l, c * NMXU + e] = jnp.where(row == _ones_row(at), 1.0, vh)
        spread.finish()
        return carry

    lax.fori_loop(0, NQ, b_proj, None)
    wait(cp_wo)

    def b_gather(g, i, accs, check):
        sub = _iota((8, T), 0)
        o = []
        for l, acc in enumerate(accs):
            at = l * DH % 8
            acc = _normalize(acc, _ones_row(at), check)
            o.append(jnp.where(sub < at, o.pop(), acc[0:8]) if l else acc[0:8])
            o += [acc[8:16], acc[16:24]]
        check[2] = check[2] + _sum(o)
        obt[i, pl.ds(pl.multiple_of(g * (BG * DH), 8), BG * DH), :] = jnp.concatenate(o, axis=0)

    def b_tile(i, g_new, g_old, spread, check):
        lane = _iota((HP // 2, T), 1)
        delta = _iota((8, T), 1) - _iota((8, T), 0)
        causal = _iota((T, T), 0) <= _iota((T, T), 1)

        def queries(h, part):
            q = qb[h, i]
            if part == 0 and i >= 2:
                q = jnp.concatenate([jnp.where(lane // HP == s, q, jnp.zeros_like(q)) for s in range(4)], axis=0)
            return _unpack(q)

        def key_rows(h):
            keys = lambda start, size: kb[h, pl.ds(start // 2, size // 2), :]
            q0 = i * T
            mid = [keys(q0 - T + r, T // 2)[:, 0:HP] if i else None for r in (0, T // 2)]
            if i < 2:
                return [keys(q0, T)[:, 0:HP], *mid]
            rows = [keys(q0, HP)]
            for s in range(1, 4):
                low = keys(q0 - WINDOW + (s - 1) * HP, HP)
                rows.append(jnp.where(lane < s * HP, low, keys(q0 + s * HP, HP)))
            rows.append(keys(q0 - WINDOW + 3 * HP, HP))
            return [jnp.concatenate(rows, axis=0), *mid]

        def park(l, z, mid1, mid2):
            for r in range(0, T, 8):
                low = z[HP + r : HP + r + 8] if i >= 2 else -jnp.inf
                pb[i, pl.ds(l * WINDOW + r, 8), :] = jnp.exp2(jnp.where(delta >= r, z[r : r + 8], low))
            if i:
                pb[i, pl.ds(l * WINDOW + T, T), :] = jnp.exp2(jnp.concatenate([mid1, mid2], axis=0))

        new = range(BG if g_new is not None else 0)
        old = range(BG if g_old is not None else 0)
        jobs = []
        for l in old:
            p = pb[i, pl.ds(l * WINDOW, T), :]
            jobs += [(l, i, jnp.where(causal, p, 0.0)), (l, i - 2, jnp.where(causal, 0.0, p))] if i >= 2 else [(l, i, p)]
        jobs += [(l, i - 1, pb[i, pl.ds(l * WINDOW + T, T), :]) for l in old if i]
        rows = [key_rows(g_new * BG + l) for l in new]
        z = [[None] * 3 for _ in new]
        accs = [None for _ in old]
        for part in range(3):
            if new and rows[0][part] is not None:
                for l in new:
                    z[l][part] = _dot(_unpack(rows[l][part]), queries(g_new * BG + l, part))
                    spread.tick(z[l][part])
            for l, j, p in jobs[part * BG : (part + 1) * BG]:
                o = _dot(vb[g_old * BG + l, j], p)
                spread.tick(o)
                accs[l] = _add(accs[l], o)
            yield
        for l in new:
            park(l, *z[l])
        if old:
            b_gather(g_old, i, accs, check)

    def b_pass(g_new, g_old, early, check):
        ticks = BG * (3 * T + (NT - 2) * (WINDOW + HP) + (0 if g_old is None else (NT - 1) * 3 * VP)) // 8
        spread, check = _Spread(early, ticks), list(check)
        for i in range(NT):
            for _ in b_tile(i, g_new, g_old, spread, check):
                pass
        spread.finish()
        return tuple(check)

    def b_exact(n, carry):
        g, i = n // NT, n % NT
        j = jnp.maximum(i - 2, 0)
        gap = (i - j) * T + _iota((3 * T, T), 1) - _iota((3 * T, T), 0)
        accs = []
        for l in range(BG):
            h = g * BG + l
            k = kb[h, pl.ds(pl.multiple_of(j * (T // 2), T // 2), 3 * T // 2), :][:, 0:HP]
            q = jnp.where(_iota((HP // 2, T), 0) < VP // 2, qb[h, i], jnp.uint32(0))
            s = jnp.where((gap >= 0) & (gap < WINDOW), _dot(_unpack(k), _unpack(q)), -jnp.inf)
            p = jnp.exp2(s - jnp.max(s, axis=0, keepdims=True))
            accs.append(_sum([_dot(vb[h, j + t], p[t * T : (t + 1) * T]) for t in range(3)]))
        b_gather(g, i, accs, list(_no_check()))
        return carry

    first = sum(EARLY_A_PROJ) + NQ * EARLY_B_PROJ
    b_pass(0, None, early_tasks(first, 0, EARLY_B_FIRST), _no_check())

    def b_attn(g, check):
        return b_pass(g, g - 1, early_tasks(first + EARLY_B_FIRST, (g - 1) * EARLY_B_PASS, EARLY_B_PASS), check)

    b_check = list(lax.fori_loop(1, H // BG, b_attn, _no_check()))

    def parked(u, n, j):
        early = A_EARLY[u % PERIOD][j]
        p = pa[u, pl.ds(j * T, T - early), :]
        if early:
            p = jnp.concatenate([p, pa_early[n, pl.ds(early_row(u % PERIOD, j), early), :]], axis=0)
        return p

    def a_couple(t, u0, b_check=None):
        first = b_check is not None
        loop = A_FIRST if first else A_LOOP
        rows = [[T - loop[j] - early[j] for j in range(NT)] for early in A_EARLY[u0 % PERIOD :][:2]]
        spread = _Spread(loop_tasks(t * A_UNROLL + u0, u0, loop), (sum(map(sum, rows)) + (BG * (min(u0 + 1, 3) + min(u0 + 2, 3)) if first else 2 * NT) * VP) // 8)
        for u in (u0, u0 + 1):
            q = _pad_rows(qa[t * A_UNROLL + u, 0:VP], HP).astype(BF16)
            acc = None
            other = b_tile(u, None, H // BG - 1, spread, b_check)
            for j0 in range(0, NT, NMXU):
                tiles = range(j0, j0 + NMXU)
                ps = [] if first else [parked(u, (t - 1) * (A_UNROLL // PERIOD) + u // PERIOD, j) for j in tiles]
                for j in tiles:
                    s = _dot(_rows(ka, j * T, rows[u % 2][j]), q)
                    pa[u, pl.ds(j * T, rows[u % 2][j]), :] = jnp.exp2(s)
                    spread.tick(s)
                for j, p in zip(tiles, ps):
                    o = _dot(va[:, pl.ds(j * T, T)], p)
                    spread.tick(o)
                    acc = _add(acc, o)
                if first:
                    next(other, None)
            if not first:
                oa[(t - 1) % (NMXU * H // A_UNROLL) * A_UNROLL + u] = acc
        spread.finish()

    def a_attn(t, carry):
        for u in range(0, A_UNROLL, 2):
            a_couple(t, u)
        return carry

    def a_last():
        for u0 in range(0, A_UNROLL, NMXU):
            accs = [None] * NMXU
            for j in range(NT):
                for u in range(u0, u0 + NMXU):
                    p = parked(u, (A_PAIRS - A_UNROLL + u) // PERIOD, j).astype(BF16)
                    accs[u - u0] = _add(accs[u - u0], _dot(va[:, pl.ds(j * T, T)], p))
            for u in range(u0, u0 + NMXU):
                oa[NMXU * H - A_UNROLL + u] = accs[u - u0]

    def a_exact(n, carry):
        s = _dot(_rows(ka, 0, S), _pad_rows(qa[n, 0:VP], HP).astype(BF16))
        oa[n % (NMXU * H)] = _dot(va[...], jnp.exp2(s - jnp.max(s, axis=0, keepdims=True)))
        return carry

    woat[...] = _pack(woa[...].T)
    wobt[...] = _pack(wob[...].T)
    for u in range(0, A_UNROLL, 2):
        a_couple(0, u, b_check)

    @pl.when(_unsafe(b_check))
    def _():
        lax.fori_loop(0, H // BG * NT, b_exact, None)

    oat = pb

    def out_copy(c, e):
        rows = pl.ds(pl.multiple_of(c * QB, QB), QB)
        dst = out_hbm.at[rows, pl.ds(max(2 * e - 1, 0) * T, obufs[e].shape[2])]
        return pltpu.make_async_copy(obufs[e].at[c % 2], dst, out_sem.at[e])

    def project(c, check):
        check = list(check)

        def gather(i, h, result):
            heads = [_normalize(oa[i * H + h + l], DH, check)[0:DH] for l in range(4)]
            o = jnp.concatenate(heads, axis=0)
            oat[i, pl.ds(h * DH, 4 * DH), :] = o
            check[2] = check[2] + jnp.sum(o.reshape(4 * DH // 8, 8, T), axis=0)
            drain(check[2], result)

        early = early_tasks(A_PAIRS - (NQ - 1) * EARLY_OUT, jnp.minimum(c, NQ - 2) * EARLY_OUT, EARLY_OUT)
        gathers = [functools.partial(gather, i, h) for h in range(0, H, 4) for i in range(NMXU)]
        cut = int(len(early) * 0.35)
        spread = _Spread(ticks=2 * D // 8 * NMXU * KT)
        spread.add(gathers, 0.0, 0.42)
        spread.add(early[:cut], 0.0, 0.42)
        spread.add(early[cut:], 0.42, 1.0)

        def part(lo, hi, i):
            if lo < D < hi:
                high = part(D, hi, i)
                return jnp.concatenate([part(lo, D, i), high], axis=0)
            if lo >= D:
                return _proj(_rows(wobt, lo - D, hi - lo), obt[c * NMXU + i], spread)
            return _proj(_rows(woat, lo, hi - lo), oat[i, pl.ds(0, D), :], spread)

        done = []
        for j in reversed(range(2 * D // T)):
            for i in range(0, NMXU, 2):
                o = jnp.concatenate([part(j * T, (j + 1) * T, i + e) for e in range(2)], axis=1)
                if len(done) >= 2:
                    drain(done[-2][-16:], o)
                done.append(o.astype(BF16).T)
                if i and j % 2 == 0 and j // 2 + 1 < len(obufs):
                    out_copy(c, j // 2 + 1).start()
                    obufs[j // 2 + 1][2, 0:8, 0:T] = o[0:8, 0:T].astype(BF16)
                obufs[(j + 1) // 2][c % 2, pl.ds(i * T, 2 * T), pl.ds((j + 1) % 2 * T if j else 0, T)] = done[-1]
        out_copy(c, 0).start()
        spread.finish()
        return tuple(check)

    def a_pass(state):
        def block(c, check):
            @pl.when(state == 0)
            def _():
                count = NMXU * H // A_UNROLL
                lax.fori_loop(c * count + 1, jnp.minimum((c + 1) * count + 1, A_PAIRS // A_UNROLL), a_attn, None)
                pl.when(c == NQ - 1)(a_last)

            @pl.when(state == 1)
            def _():
                lax.fori_loop(c * NMXU * H, (c + 1) * NMXU * H, a_exact, None)

            @pl.when(c > 0)
            def _():
                wait([out_copy(c - 1, e) for e in range(len(obufs))])

            return project(c, check)

        check = lax.fori_loop(0, NQ, block, _no_check())
        wait([out_copy(NQ - 1, e) for e in reversed(range(len(obufs)))])
        return jnp.where((state == 0) & _unsafe(check), 1, 2)

    lax.while_loop(lambda state: state < 2, a_pass, 0)


@jax.jit
def pallas_concat_heads__grouped_kv_mqa__sliding_block__prompt_kernel(
    A_x: jax.Array,
    A_wq: jax.Array,
    A_wk: jax.Array,
    A_wv: jax.Array,
    A_wo: jax.Array,
    B_x: jax.Array,
    B_wqkv: jax.Array,
    B_wo: jax.Array,
):
    assert A_x.shape == (1, S, D) and B_x.shape == (1, S, D)
    vmem = pltpu.VMEM
    out = pl.pallas_call(
        _kernel,
        out_shape=jax.ShapeDtypeStruct((S, 2 * D), BF16),
        in_specs=[pl.BlockSpec(memory_space=pl.ANY)] * 8,
        out_specs=pl.BlockSpec(memory_space=pl.ANY),
        scratch_shapes=[
            vmem((NQ, D, QB), BF16),
            vmem((D, D), BF16),
            vmem((D, D), BF16),
            vmem((NQ, D, QB), BF16),
            vmem((D, 3 * D), BF16),
            vmem((D, D), BF16),
            vmem((D // 2, D), U32),
            vmem((3 * D // 2, D), U32),
            vmem((D // 2, D), U32),
            vmem((D // 2, D), U32),
            vmem((A_PAIRS, HP, T), F32),
            vmem((S // 2, HP), U32),
            vmem((DH, sum(A_EARLY_MAX), T), F32),
            vmem((sum(A_LOOP) // 16, 7 * DH // 2, 8, T), F32),
            vmem((A_UNROLL // 2, sum(A_LOOP) // 16, 4, 8, T), F32),
            vmem((VP, S), F32),
            vmem((A_UNROLL, S, T), F32),
            vmem((A_PAIRS // PERIOD, sum(map(sum, A_EARLY)), T), F32),
            vmem((NMXU * H, VP, T), F32),
            vmem((H, NT, HP // 2, T), U32),
            vmem((H, S // 2, T), U32),
            vmem((H, NT, VP, T), F32),
            vmem((NT, BG * WINDOW, T), F32),
            vmem((NT, D, T), F32),
            [vmem((2, QB, T), BF16)] + [vmem((3, QB, 2 * T), BF16)] * (D // T),
            vmem((128, 8, T), U32),
            vmem((DH, D), BF16),
            vmem((DH, D), BF16),
            pltpu.SemaphoreType.DMA((6 + 2 * NQ,)),
            pltpu.SemaphoreType.DMA((D // T + 1,)),
        ],
        compiler_params=pltpu.CompilerParams(vmem_limit_bytes=125 * 1024 * 1024),
        name="mqa_swa_fused",
    )(A_x[0].T, A_wq, A_wk.T, A_wv.T, A_wo, B_x[0].T, B_wqkv, B_wo)
    return out[None]
```
